```python
import os as _os
_os.environ.setdefault("JAX_PLATFORMS", "cpu")
import jax
import jax.numpy as jnp

def _softmax(x, axis=-1):
    return jax.nn.softmax(x, axis=axis)
def _gelu(x):
    return jax.nn.gelu(x, approximate=True)
def _silu(x):
    return jax.nn.silu(x)
def _sigmoid(x):
    return jax.nn.sigmoid(x)
def _layernorm(x, axis=-1, eps=1e-5):
    m = jnp.mean(x, axis=axis, keepdims=True)
    v = jnp.var(x, axis=axis, keepdims=True)
    return (x - m) / jnp.sqrt(v + eps)
def _scatter_add(tgt, idx, src, axis=0):
    return tgt.at[idx].add(src)
def _segment_sum(src, seg, n):
    return jax.ops.segment_sum(src, seg, n)
class _Rng:
    def __init__(self, key):
        self._k = key
    def _next(self):
        self._k, sub = jax.random.split(self._k)
        return sub
    def normal(self, shape):
        return jax.random.normal(self._next(), shape, dtype=jnp.bfloat16)
    def randint(self, lo, hi, shape):
        return jax.random.randint(self._next(), shape, lo, hi, dtype=jnp.int32)
    def uniform(self, shape, lo=0.0, hi=1.0):
        return jax.random.uniform(self._next(), shape, jnp.bfloat16, lo, hi)
    def permutation(self, n):
        return jax.random.permutation(self._next(), n)


kernel_name = 'concat_heads__spectral_gfnet__mha_block__prompt'

def setup_inputs():
    _rng = _Rng(jax.random.key(int.from_bytes(__import__("os").urandom(4), "little")))
    _w = (lambda a: (lambda t: t.astype(jnp.bfloat16) if jnp.issubdtype(t.dtype, jnp.floating) else t)(jnp.asarray(a)))
    def _A_setup():
        B, S, D = 1, 2048, 576
        Df = D // 2 + 1
        return {
            "x": _w((lambda *s: _rng.normal(s) * 0.05)(B, S, D)),
            "w_r": _w((lambda *s: _rng.normal(s) * 0.05)(S, Df) * 0.02),
            "w_i": _w((lambda *s: _rng.normal(s) * 0.05)(S, Df) * 0.02),
        }
    _A_in = _A_setup()

    def _B_setup():
        B, S, D, H = 1, 2048, 576, 32
        return {
            "x": _w((lambda *s: _rng.normal(s) * 0.1)(B, S, D)),
            "wqkv": _w((lambda *s: _rng.normal(s) * 0.1)(D, 3 * D)),
            "wo": _w((lambda *s: _rng.normal(s) * 0.05)(D, D)),
        }
    _B_in = _B_setup()

    return {
        "A_x": _A_in["x"],
        "A_w_r": _A_in["w_r"],
        "A_w_i": _A_in["w_i"],
        "B_x": _B_in["x"],
        "B_wqkv": _B_in["wqkv"],
        "B_wo": _B_in["wo"],
    }

def reference(A_x, A_w_r, A_w_i, B_x, B_wqkv, B_wo):
    def _A_ref(x, w_r, w_i):
        B, S, D = x.shape
        X = (lambda x, axes=(-2,-1): jnp.fft.rfft2(x.astype(jnp.float32), axes=axes))(x, axes=(-2, -1))
        W = w_r + 1j * w_i
        X = X * W
        y = (lambda x, s, axes=(-2,-1): jnp.fft.irfft2(x, s=s, axes=axes).astype(jnp.bfloat16))(X, (S, D), axes=(-2, -1))
        return y

    def _B_ref(x, wqkv, wo):
        B, S, D = x.shape
        H = 32
        Dh = D // H
        qkv = (lambda x, *d: x.transpose(*d))((x @ wqkv).reshape(B, S, 3, H, Dh), 2, 0, 3, 1, 4)
        q, k, v = qkv[0], qkv[1], qkv[2]
        scores = jnp.einsum("bhqd,bhkd->bhqk", q, k) * (Dh ** -0.5)
        p = _softmax(scores, axis=-1)
        o = jnp.einsum("bhqk,bhkd->bhqd", p, v)
        return (lambda x, *d: x.transpose(*d))(o, 0, 2, 1, 3).reshape(B, S, D) @ wo

    a = _A_ref(A_x, A_w_r, A_w_i)
    b = _B_ref(B_x, B_wqkv, B_wo)
    return jnp.concatenate([a, b], axis=-1)
```

```python
import functools

import numpy as np
import jax
import jax.numpy as jnp
from jax.experimental import pallas as pl
from jax.experimental.pallas import tpu as pltpu

S, D, H, DH = 2048, 576, 32, 18
DF = D // 2 + 1
FP = 384
HPG = 7
NG = 5
VR = 32
N1, N2 = 16, 128
MQ = 256
KC = 256
WM = 0.3
NQ = S // MQ
NC = S // KC
QSCALE = float(DH ** -0.5 * np.log2(np.e))
F32 = jnp.float32
BF16 = jnp.bfloat16


def _tables():
    d = np.arange(D)[:, None].astype(np.float64)
    l = np.arange(DF)[None, :].astype(np.float64)
    ang = 2.0 * np.pi * ((d * l) % D) / D
    fd = np.zeros((D, 2 * FP), np.float64)
    fd[:, :DF] = np.cos(ang)
    fd[:, FP:FP + DF] = -np.sin(ang)
    c = np.full((DF,), 2.0)
    c[0] = 1.0
    c[DF - 1] = 1.0
    fi = np.zeros((2 * FP, 640), np.float64)
    fi[:DF, :D] = (c[:, None] * np.cos(ang.T)) / (S * D)
    si = -(c[:, None] * np.sin(ang.T)) / (S * D)
    si[0, :] = 0.0
    si[DF - 1, :] = 0.0
    fi[FP:FP + DF, :D] = si
    k2 = np.arange(N2)[:, None]
    n2 = np.arange(N2)[None, :]
    g = np.zeros((N1, 2 * N2, 2 * N2), np.float64)
    for n1 in range(N1):
        th = 2.0 * np.pi * ((k2 * (n1 + N1 * n2)) % S) / S
        cr, ci = np.cos(th), -np.sin(th)
        g[n1, :N2, :N2] = cr
        g[n1, :N2, N2:] = -ci
        g[n1, N2:, :N2] = ci
        g[n1, N2:, N2:] = cr
    hh = np.transpose(g, (0, 2, 1))
    return (fd.astype(np.float32), fi.astype(np.float32),
            g.astype(np.float32), np.ascontiguousarray(hh).astype(np.float32))


def _cmul_const(xr, xi, k, n, sign):
    k = k % n
    if k == 0:
        return xr, xi
    if 4 * k == n:
        return (-xi, xr) if sign > 0 else (xi, -xr)
    if 2 * k == n:
        return -xr, -xi
    if 4 * k == 3 * n:
        return (xi, -xr) if sign > 0 else (-xi, xr)
    c = float(np.cos(2 * np.pi * k / n))
    s = float(sign * np.sin(2 * np.pi * k / n))
    if abs(abs(c) - abs(s)) < 1e-12:
        if c * s > 0:
            return (xr - xi) * c, (xr + xi) * c
        return (xr + xi) * c, (xi - xr) * c
    return xr * c - xi * s, xr * s + xi * c


def _fft(xs, sign):
    n = len(xs)
    if n == 1:
        return xs
    ev = _fft(xs[0::2], sign)
    od = _fft(xs[1::2], sign)
    out = [None] * n
    for k in range(n // 2):
        tr, ti = _cmul_const(od[k][0], od[k][1], k, n, sign)
        er, ei = ev[k]
        out[k] = (er + tr, ei + ti)
        out[k + n // 2] = (er - tr, ei - ti)
    return out


def _kernel(ax_ref, wr_ref, wi_ref, bx_ref, wqkv_ref, wo_ref,
            fd_ref, fi_ref, g_ref, h_ref, o_ref,
            y_s, t_s, wr_s, wi_s,
            wq_s, wk_s, wvt_s, wo_s, k_s, qt_s, vt_s, ot_s, sa, sb):
    nt = (((1,), (1,)), ((), ()))

    RB = 256
    for r in range(S // RB):
        yy = jnp.dot(ax_ref[r * RB:(r + 1) * RB, :], fd_ref[...], preferred_element_type=F32)
        for j in range(6):
            y_s[j, r * RB:(r + 1) * RB, :] = yy[:, j * 128:(j + 1) * 128]
    wr_s[:, 256:] = jnp.zeros((S, FP - 256), F32)
    wi_s[:, 256:] = jnp.zeros((S, FP - 256), F32)
    wr_s[:, :DF] = wr_ref[...].astype(F32)
    wi_s[:, :DF] = wi_ref[...].astype(F32)

    for n1 in range(N1):
        yn = [y_s[j, pl.ds(n1, N2, stride=N1), :] for j in range(6)]
        rhs = jnp.concatenate([jnp.concatenate(yn[:3], axis=1),
                               jnp.concatenate(yn[3:], axis=1)], axis=0).astype(BF16)
        t_s[n1] = jnp.dot(g_ref[n1], rhs, preferred_element_type=F32)

    def fft_body(rc, carry):
        r0 = pl.multiple_of(rc * 8, 8)
        for j in range(FP // 128):
            ls = slice(j * 128, (j + 1) * 128)
            xs = [(t_s[n1, pl.ds(r0, 8), ls], t_s[n1, pl.ds(N2 + r0, 8), ls])
                  for n1 in range(N1)]
            xf = _fft(xs, -1)
            us = []
            for k1 in range(N1):
                wr = wr_s[pl.ds(k1 * N2 + r0, 8), ls]
                wi = wi_s[pl.ds(k1 * N2 + r0, 8), ls]
                xr, xi = xf[k1]
                us.append((xr * wr - xi * wi, xr * wi + xi * wr))
            ys = _fft(us, +1)
            for n1 in range(N1):
                t_s[n1, pl.ds(r0, 8), ls] = ys[n1][0]
                t_s[n1, pl.ds(N2 + r0, 8), ls] = ys[n1][1]
        return carry
    jax.lax.fori_loop(0, N2 // 8, fft_body, 0)

    for n1 in range(N1):
        z = jnp.dot(h_ref[n1], t_s[n1].astype(BF16), preferred_element_type=F32)
        for j in range(3):
            y_s[j, pl.ds(n1, N2, stride=N1), :] = z[:N2, j * 128:(j + 1) * 128]
            y_s[3 + j, pl.ds(n1, N2, stride=N1), :] = z[N2:, j * 128:(j + 1) * 128]

    GW = HPG * DH
    wq_s[...] = jnp.zeros(wq_s.shape, BF16)
    wk_s[...] = jnp.zeros(wk_s.shape, BF16)
    for g in range(NG):
        w = min(GW, D - g * GW)
        wq_s[:, g * 128:g * 128 + w] = wqkv_ref[:, g * GW:g * GW + w]
        wk_s[:, g * 128:g * 128 + w] = wqkv_ref[:, D + g * GW:D + g * GW + w]
    wvt = wqkv_ref[:, 2 * D:].astype(F32).T
    wof = wo_ref[...].astype(F32)
    wvt_s[...] = jnp.zeros(wvt_s.shape, F32)
    wo_s[...] = jnp.zeros(wo_s.shape, F32)
    for h in range(H):
        wvt_s[h * VR:h * VR + DH, :] = wvt[h * DH:(h + 1) * DH, :]
        wo_s[h * VR:h * VR + DH, :] = wof[h * DH:(h + 1) * DH, :]

    x = bx_ref[...]
    kk = jnp.dot(x, wk_s[...], preferred_element_type=F32).astype(BF16)
    for g in range(NG):
        k_s[g] = kk[:, g * 128:(g + 1) * 128]
    wqt = wq_s[...].astype(F32).T.astype(BF16)
    for qb in range(NQ):
        xq = bx_ref[qb * MQ:(qb + 1) * MQ, :]
        qt = jax.lax.dot_general(wqt, xq, nt, preferred_element_type=F32)
        qt_s[qb] = (qt * QSCALE).astype(BF16)
    vt = jax.lax.dot_general(wvt_s[...].astype(BF16), x, nt, preferred_element_type=F32)
    row = jax.lax.broadcasted_iota(jnp.int32, vt.shape, 0)
    vt = jnp.where((row % VR) == DH, 1.0, vt)
    vt_s[...] = vt.astype(BF16)

    def get_qm(t):
        h = t // NQ
        qb = t % NQ
        g = h // HPG
        j = h % HPG
        qg = qt_s[qb, pl.ds(pl.multiple_of(g * 128, 128), 128), :]
        r = jax.lax.broadcasted_iota(jnp.int32, qg.shape, 0)
        qm = jnp.where((r >= j * DH) & (r < j * DH + DH), qg, jnp.zeros_like(qg))
        return g, qm

    def step(t_qk, s_w, t_sm, s_r):
        st = {}
        qk_ops = []
        if t_qk is not None:
            g, qm = get_qm(t_qk)

            def qk_c(c):
                s_w[c * KC:(c + 1) * KC, :] = jnp.dot(
                    k_s[g, c * KC:(c + 1) * KC, :], qm, preferred_element_type=F32)
            qk_ops = [functools.partial(qk_c, c) for c in range(NC)]
        sm_ops = []
        if t_sm is not None:
            h = t_sm // NQ
            qb = t_sm % NQ
            hv = pl.multiple_of(h * VR, VR)
            st["mx"] = None
            st["acc"] = None

            def mx_c(c):
                m = jnp.max(s_r[c * KC:(c + 1) * KC, :].reshape(KC // 8, 8, MQ), axis=0)
                st["mx"] = m if st["mx"] is None else jnp.maximum(st["mx"], m)
                if c == NC - 1:
                    st["m"] = jnp.max(st["mx"], axis=0, keepdims=True)

            def ex_c(c):
                p = jnp.exp2(s_r[c * KC:(c + 1) * KC, :] - st["m"]).astype(BF16)
                v = vt_s[pl.ds(hv, VR), c * KC:(c + 1) * KC]
                o = jnp.dot(v, p, preferred_element_type=F32)
                st["acc"] = o if st["acc"] is None else st["acc"] + o
                if c == NC - 1:
                    acc = st["acc"]
                    l = acc[DH:DH + 1, :]
                    ot_s[qb, pl.ds(hv, VR), :] = (acc * (1.0 / l)).astype(BF16)
            sm_ops = ([(WM, functools.partial(mx_c, c)) for c in range(NC)]
                      + [(1.0, functools.partial(ex_c, c)) for c in range(NC)])
        tot = sum(w for w, _ in sm_ops)
        k = 0
        cum = 0.0
        for i, q in enumerate(qk_ops):
            q()
            while k < len(sm_ops) and cum + sm_ops[k][0] <= tot * (i + 1) / len(qk_ops) + 1e-9:
                cum += sm_ops[k][0]
                sm_ops[k][1]()
                k += 1
        while k < len(sm_ops):
            sm_ops[k][1]()
            k += 1

    T = H * NQ
    step(0, sa, None, None)

    def body(i, c):
        t = 2 * i
        step(t + 1, sb, t, sa)
        step(t + 2, sa, t + 1, sb)
        return c
    jax.lax.fori_loop(0, T // 2 - 1, body, 0)
    step(T - 1, sb, T - 2, sa)
    step(None, None, T - 1, sb)

    wot = wo_s[...].T.astype(BF16)
    for qb in range(NQ):
        rows = slice(qb * MQ, (qb + 1) * MQ)
        ot = jnp.dot(wot, ot_s[qb], preferred_element_type=F32)
        otp = jnp.concatenate([jnp.zeros((64, MQ), F32), ot], axis=0)
        bp = otp.T
        yr = jnp.concatenate([y_s[j, rows, :] for j in range(6)], axis=1).astype(BF16)
        a = jnp.dot(yr, fi_ref[...], preferred_element_type=F32)
        o_ref[rows, 0:512] = a[:, 0:512].astype(BF16)
        o_ref[rows, 512:640] = (a[:, 512:640] + bp[:, 0:128]).astype(BF16)
        o_ref[rows, 640:1152] = bp[:, 128:640].astype(BF16)


@jax.jit
def pallas_concat_heads__spectral_gfnet__mha_block__prompt_kernel(
    A_x: jax.Array,
    A_w_r: jax.Array,
    A_w_i: jax.Array,
    B_x: jax.Array,
    B_wqkv: jax.Array,
    B_wo: jax.Array,
):
    fd, fi, g, hh = _tables()
    fd = jnp.asarray(fd, BF16)
    fi = jnp.asarray(fi, BF16)
    g = jnp.asarray(g, BF16)
    hh = jnp.asarray(hh, BF16)
    out = pl.pallas_call(
        _kernel,
        out_shape=jax.ShapeDtypeStruct((S, 2 * D), BF16),
        scratch_shapes=[
            pltpu.VMEM((6, S, 128), F32),
            pltpu.VMEM((N1, 2 * N2, FP), F32),
            pltpu.VMEM((S, FP), F32),
            pltpu.VMEM((S, FP), F32),
            pltpu.VMEM((D, NG * 128), BF16),
            pltpu.VMEM((D, NG * 128), BF16),
            pltpu.VMEM((H * VR, D), F32),
            pltpu.VMEM((H * VR, D), F32),
            pltpu.VMEM((NG, S, 128), BF16),
            pltpu.VMEM((NQ, NG * 128, MQ), BF16),
            pltpu.VMEM((H * VR, S), BF16),
            pltpu.VMEM((NQ, H * VR, MQ), BF16),
            pltpu.VMEM((S, MQ), F32),
            pltpu.VMEM((S, MQ), F32),
        ],
        compiler_params=pltpu.CompilerParams(vmem_limit_bytes=110 * 1024 * 1024),
    )(A_x.reshape(S, D), A_w_r, A_w_i, B_x.reshape(S, D), B_wqkv, B_wo, fd, fi, g, hh)
    return out.reshape(1, S, 2 * D)
```

```python
import functools

import numpy as np
import jax
import jax.numpy as jnp
from jax.experimental import pallas as pl
from jax.experimental.pallas import tpu as pltpu

S, D, H, DH = 2048, 576, 32, 18
DF = D // 2 + 1
DH2 = D // 2
TR = 80
NT = 4
HPG = 7
NG = 5
GW = HPG * DH
VR = 32
N1, N2 = 16, 128
MQ = 512
KC = 128
WM = 0.3
UNR = 4
NQ = S // MQ
NC = S // KC
PB = 256
NPB = S // PB
AB = 512
NAB = S // AB
OB = 256
NOB = S // OB
SL_A1, SL_FF, SL_M1, SL_M2, SL_FI = 0, 11, 24, 28, 48
QSCALE = float(DH ** -0.5 * np.log2(np.e))
F32 = jnp.float32
BF16 = jnp.bfloat16


def _tables():
    d = np.arange(DH2)[None, :].astype(np.float64)
    fa = np.zeros((NT, 2 * TR, DH2), np.float64)
    fi2 = np.zeros((2, DH2, 4 * TR), np.float64)
    for c in range(NT):
        p, half = c // 2, c % 2
        l = p + 2 * (TR * half + np.arange(TR))
        valid = (l <= DF - 1).astype(np.float64)[:, None]
        lf = l[:, None].astype(np.float64)
        ang = 2.0 * np.pi * ((lf * d) % D) / D
        fa[c, :TR] = np.cos(ang) * valid
        fa[c, TR:] = -np.sin(ang) * valid
        cl = np.where((l == 0) | (l == DF - 1), 1.0, 2.0)[:, None] * valid
        im_ok = ((l != 0) & (l != DF - 1)).astype(np.float64)[:, None]
        fi2[p, :, half * 2 * TR:half * 2 * TR + TR] = (cl * np.cos(ang)).T / (S * D)
        fi2[p, :, half * 2 * TR + TR:(half + 1) * 2 * TR] = (-cl * im_ok * np.sin(ang)).T / (S * D)
    n2 = np.arange(N2)[:, None]
    k2 = np.arange(N2)[None, :]
    cf = np.zeros((N1, 2 * N2, 2 * N2), np.float64)
    for k1 in range(N1):
        th = 2.0 * np.pi * ((n2 * (k1 + N1 * k2)) % S) / S
        cr, ci = np.cos(th), -np.sin(th)
        cf[k1, :N2, :N2] = cr
        cf[k1, :N2, N2:] = ci
        cf[k1, N2:, :N2] = -ci
        cf[k1, N2:, N2:] = cr
    cb = np.ascontiguousarray(np.transpose(cf, (0, 2, 1)))
    return (fa.astype(np.float32), fi2.astype(np.float32),
            cf.astype(np.float32), cb.astype(np.float32))


def _cmul_const(xr, xi, k, n, sign):
    k = k % n
    if k == 0:
        return xr, xi
    if 4 * k == n:
        return (-xi, xr) if sign > 0 else (xi, -xr)
    if 2 * k == n:
        return -xr, -xi
    if 4 * k == 3 * n:
        return (xi, -xr) if sign > 0 else (-xi, xr)
    c = float(np.cos(2 * np.pi * k / n))
    s = float(sign * np.sin(2 * np.pi * k / n))
    if abs(abs(c) - abs(s)) < 1e-12:
        if c * s > 0:
            return (xr - xi) * c, (xr + xi) * c
        return (xr + xi) * c, (xi - xr) * c
    return xr * c - xi * s, xr * s + xi * c


def _fft(xs, sign):
    n = len(xs)
    if n == 1:
        return xs
    ev = _fft(xs[0::2], sign)
    od = _fft(xs[1::2], sign)
    out = [None] * n
    for k in range(n // 2):
        tr, ti = _cmul_const(od[k][0], od[k][1], k, n, sign)
        er, ei = ev[k]
        out[k] = (er + tr, ei + ti)
        out[k + n // 2] = (er - tr, ei - ti)
    return out


def _kernel(axt_hbm, wrt_hbm, wit_hbm, bxt_hbm, wqkv_hbm, wo_hbm,
            fa_hbm, fi_hbm, cf_hbm, cb_hbm, o_hbm,
            axt, wrt, wit, bxt, wqkv, wo, fa, fi2, cf, cb, sems, bsem, osem, osem2,
            xs_s, y_s, t_s, u_s, wn_s, wq_s, yb_s, at_s,
            wl_s, wl_b, wot_s, k_s, qt_s, vt_s, ot_s, sa, sb, ob_s):
    names = ["wqkv", "wrt", "wit", "axt", "fa", "cf", "cb", "fi", "wo"]
    srcs = [wqkv_hbm, wrt_hbm, wit_hbm, axt_hbm, fa_hbm, cf_hbm, cb_hbm, fi_hbm, wo_hbm]
    dsts = [wqkv, wrt, wit, axt, fa, cf, cb, fi2, wo]
    cp = {n_: pltpu.make_async_copy(s_, d_, sems.at[i])
          for i, (n_, s_, d_) in enumerate(zip(names, srcs, dsts))}

    def bx_copy(i):
        cols = pl.ds(pl.multiple_of(i * PB, PB), PB)
        return pltpu.make_async_copy(bxt_hbm.at[:, cols], bxt.at[:, cols], bsem.at[i])

    cp["wqkv"].start()
    bx_copy(0).start()

    cp["wqkv"].wait()
    for i_ in range(1, NPB):
        bx_copy(i_).start()
    for n_ in names[1:]:
        cp[n_].start()
    wt = wqkv[...].astype(F32).T
    wl_s[...] = jnp.zeros(wl_s.shape, F32)
    for g in range(NG):
        w = min(GW, D - g * GW)
        wl_s[g * 128:g * 128 + w, :] = wt[g * GW:g * GW + w, :]
        wl_s[640 + g * 128:640 + g * 128 + w, :] = wt[D + g * GW:D + g * GW + w, :]
    wl_s[1280:1280 + D, :] = wt[2 * D:, :]
    wl_b[...] = wl_s[...].astype(BF16)

    def proj_block(cbk):
        bx_copy(cbk).wait()
        c0 = pl.multiple_of(cbk * PB, PB)
        cols = pl.ds(c0, PB)
        pr = jnp.dot(wl_b[...], bxt[:, cols], preferred_element_type=F32)
        qt_s[(cbk * PB) // MQ, :, pl.ds(pl.multiple_of((cbk * PB) % MQ, PB), PB)] = (
            pr[:640, :] * QSCALE).astype(BF16)
        kt = pr[640:1280, :].T.astype(BF16)
        for g in range(NG):
            k_s[g, cols, :] = kt[:, g * 128:(g + 1) * 128]
        vt = pr[1280:, :]
        pad = jnp.concatenate([jnp.ones((1, PB), F32), jnp.zeros((VR - DH - 1, PB), F32)], axis=0)
        for h in range(H):
            blk = jnp.concatenate([vt[h * DH:(h + 1) * DH, :], pad], axis=0)
            vt_s[h * VR:(h + 1) * VR, cols] = blk.astype(BF16)

    def wperm1(c):
        l0 = pl.multiple_of(c * 128, 128)
        hi = pltpu.bitcast(wrt[:, pl.ds(l0, 128)].astype(F32), jnp.int32)
        lo = pltpu.bitcast(wit[:, pl.ds(l0, 128)].astype(F32), jnp.int32)
        blk = hi | jax.lax.shift_right_logical(lo, 16)
        blk = jnp.concatenate([blk, jnp.zeros((384 - DF, 128), jnp.int32)], axis=0)
        bt = blk.T
        for j in range(3):
            wn_s[j, pl.ds(l0, 128), :] = bt[:, j * 128:(j + 1) * 128]

    def wperm2(k1):
        for j in range(3):
            wq_s[k1, j * 128:(j + 1) * 128, :] = wn_s[j, pl.ds(k1, N2, stride=N1), :].T

    HP = NPB // 2

    def proj_a(i, carry):
        proj_block(i)
        return carry
    jax.lax.fori_loop(0, HP, proj_a, 0)

    cp["wrt"].wait()
    cp["wit"].wait()
    cp["axt"].wait()

    def proj_b(i, carry):
        proj_block(HP + i)
        for cc in range(N1 // HP):
            wperm1(i * (N1 // HP) + cc)
        cols = pl.ds(pl.multiple_of(i * (S // HP), S // HP), S // HP)
        x0 = axt[0:DH2, cols].astype(F32)
        x1 = axt[DH2:D, cols].astype(F32)
        xs_s[0, :, cols] = (x0 + x1).astype(BF16)
        xs_s[1, :, cols] = (x0 - x1).astype(BF16)
        return carry
    jax.lax.fori_loop(0, HP, proj_b, 0)

    cp["wo"].wait()
    cp["fa"].wait()
    cp["cf"].wait()
    cp["cb"].wait()
    cp["fi"].wait()

    def task_ops(c):
        p = c // 2
        half = c % 2
        sched = {}

        def put(slot, op):
            sched.setdefault(slot, []).append(op)

        def a1(j):
            cols = slice(j * 256, (j + 1) * 256)
            y_s[:, cols] = jnp.dot(fa[c], xs_s[p, :, cols], preferred_element_type=F32)
        for j in range(8):
            put(SL_A1 + j, functools.partial(a1, j))

        def ffwd(rc):
            rr = rc * 8
            xs = [(y_s[rr:rr + 8, n1 * 128:(n1 + 1) * 128],
                   y_s[TR + rr:TR + rr + 8, n1 * 128:(n1 + 1) * 128]) for n1 in range(N1)]
            out = _fft(xs, -1)
            for k1 in range(N1):
                t_s[k1, rr:rr + 8, 0:128] = out[k1][0]
                t_s[k1, rr:rr + 8, 128:256] = out[k1][1]
        for rc in range(TR // 8):
            put(SL_FF + rc, functools.partial(ffwd, rc))

        def mid1(k1):
            xk = jnp.dot(t_s[k1].astype(BF16), cf[k1], preferred_element_type=F32)
            xr, xi = xk[:, :128], xk[:, 128:]
            r0 = p + 2 * TR * half
            wp = wq_s[k1, pl.ds(r0, TR, stride=2), :]
            wr = pltpu.bitcast(wp & jnp.int32(-65536), F32)
            wi = pltpu.bitcast(jax.lax.shift_left(wp, 16), F32)
            u_s[k1] = jnp.concatenate([xr * wr - xi * wi, xr * wi + xi * wr], axis=1).astype(BF16)

        def mid2(k1):
            vk = jnp.dot(u_s[k1], cb[k1], preferred_element_type=F32)
            y_s[0:TR, k1 * 128:(k1 + 1) * 128] = vk[:, :128]
            y_s[TR:2 * TR, k1 * 128:(k1 + 1) * 128] = vk[:, 128:]
        for k1 in range(N1):
            put(SL_M1 + k1, functools.partial(mid1, k1))
            put(SL_M2 + k1, functools.partial(mid2, k1))

        def finv(rc):
            rr = rc * 8
            xs = [(y_s[rr:rr + 8, k1 * 128:(k1 + 1) * 128],
                   y_s[TR + rr:TR + rr + 8, k1 * 128:(k1 + 1) * 128]) for k1 in range(N1)]
            out = _fft(xs, +1)
            b0 = pl.multiple_of(half * 2 * TR + rr, 8)
            b1 = pl.multiple_of(half * 2 * TR + TR + rr, 8)
            for n1 in range(N1):
                yb_s[p, pl.ds(b0, 8), n1 * 128:(n1 + 1) * 128] = out[n1][0]
                yb_s[p, pl.ds(b1, 8), n1 * 128:(n1 + 1) * 128] = out[n1][1]
        for rc in range(TR // 8):
            put(SL_FI + rc, functools.partial(finv, rc))
        return sched

    def out_copy_a(j):
        rows = pl.ds(pl.multiple_of(j * AB, AB), AB)
        return pltpu.make_async_copy(ob_s.at[rows, pl.ds(0, 512)], o_hbm.at[rows, pl.ds(0, 512)],
                                     osem.at[j])

    def out_copy_b(ob):
        rows = pl.ds(pl.multiple_of(ob * OB, OB), OB)
        return pltpu.make_async_copy(ob_s.at[rows, pl.ds(512, 640)], o_hbm.at[rows, pl.ds(512, 640)],
                                     osem2.at[ob])

    def a7_ops(j):
        def one(q):
            cols = pl.ds(pl.multiple_of(j * AB + q * 128, 128), 128)
            e = jnp.dot(fi2[0], yb_s[0, :, cols].astype(BF16), preferred_element_type=F32)
            o = jnp.dot(fi2[1], yb_s[1, :, cols].astype(BF16), preferred_element_type=F32)
            ao = jnp.concatenate([e + o, e - o], axis=0)
            ob_s[cols, 0:512] = ao[:512].T.astype(BF16)
            at_s[:, cols] = ao[512:]
        return {4 + 14 * q: [functools.partial(one, q)] for q in range(AB // 128)}

    def get_qm(t):
        h = t // NQ
        qb = t % NQ
        g = h // HPG
        j = h % HPG
        qg = qt_s[qb, pl.ds(pl.multiple_of(g * 128, 128), 128), :]
        r = jax.lax.broadcasted_iota(jnp.int32, qg.shape, 0)
        qm = jnp.where((r >= j * DH) & (r < j * DH + DH), qg, jnp.zeros_like(qg))
        return g, qm

    def step(t_qk, s_w, t_sm, s_r, m_in, want_m, extra={}):
        st = {}
        qk_ops = []
        if t_qk is not None:
            g, qm = get_qm(t_qk)
            st["mw"] = None

            def qk_c(c):
                s = jnp.dot(k_s[g, c * KC:(c + 1) * KC, :], qm, preferred_element_type=F32)
                s_w[c * KC:(c + 1) * KC, :] = s
                if want_m:
                    m = jnp.max(s.reshape(KC // 8, 8, MQ), axis=0)
                    st["mw"] = m if st["mw"] is None else jnp.maximum(st["mw"], m)
            qk_ops = [functools.partial(qk_c, c) for c in range(NC)]
        sm_ops = []
        if t_sm is not None:
            h = t_sm // NQ
            qb = t_sm % NQ
            hv = h * VR if isinstance(h, int) else pl.multiple_of(h * VR, VR)
            st["mx"] = None
            st["acc"] = None
            st["m"] = m_in

            def mx_c(c):
                m = jnp.max(s_r[c * KC:(c + 1) * KC, :].reshape(KC // 8, 8, MQ), axis=0)
                st["mx"] = m if st["mx"] is None else jnp.maximum(st["mx"], m)
                if c == NC - 1:
                    st["m"] = jnp.max(st["mx"], axis=0, keepdims=True)

            def ex_c(c):
                p = jnp.exp2(s_r[c * KC:(c + 1) * KC, :] - st["m"]).astype(BF16)
                v = vt_s[pl.ds(hv, VR), c * KC:(c + 1) * KC]
                o = jnp.dot(v, p, preferred_element_type=F32)
                st["acc"] = o if st["acc"] is None else st["acc"] + o
                if c == NC - 1:
                    acc = st["acc"]
                    l = acc[DH:DH + 1, :]
                    ot_s[qb, pl.ds(hv, VR), :] = acc * (1.0 / l)
            if m_in is None:
                sm_ops = [(WM, functools.partial(mx_c, c)) for c in range(NC)]
            sm_ops += [(1.0, functools.partial(ex_c, c)) for c in range(NC)]
        tot = sum(w for w, _ in sm_ops)
        k = 0
        cum = 0.0
        for i, q in enumerate(qk_ops):
            q()
            while k < len(sm_ops) and cum + sm_ops[k][0] <= tot * (i + 1) / len(qk_ops) + 1e-9:
                cum += sm_ops[k][0]
                sm_ops[k][1]()
                k += 1
            for op in extra.get(i, ()):
                op()
        while k < len(sm_ops):
            sm_ops[k][1]()
            k += 1
        if want_m:
            return jnp.max(st["mw"], axis=0, keepdims=True)

    T = H * NQ
    bufs = [sa, sb]
    m0 = step(0, sa, None, None, None, True,
              {k1: [functools.partial(wperm2, k1)] for k1 in range(N1)})
    nb = (T - 1) // UNR

    def make_body(extra_fn, post_fn=None):
        def body(i, m):
            t = UNR * i
            ex = extra_fn(i) if extra_fn is not None else {}
            mm = None
            for u in range(UNR):
                part = {sl - u * NC: ops for sl, ops in ex.items() if u * NC <= sl < (u + 1) * NC}
                mm = step(t + u + 1, bufs[(u + 1) % 2], t + u, bufs[u % 2],
                          m if u == 0 else None, u == UNR - 1, part)
            if post_fn is not None:
                post_fn(i)
            return mm
        return body

    m = jax.lax.fori_loop(0, NT, make_body(task_ops), m0)
    m = jax.lax.fori_loop(NT, NT + NAB, make_body(lambda i: a7_ops(i - NT),
                                                  lambda i: out_copy_a(i - NT).start()), m)
    m = jax.lax.fori_loop(NT + NAB, nb, make_body(None), m)
    t0 = nb * UNR
    def prep_wot():
        wot_s[...] = wo[...].astype(F32).T.astype(BF16)

    for t in range(t0, T):
        u = t - t0
        step(t + 1 if t + 1 < T else None, bufs[(u + 1) % 2], t, bufs[u % 2],
             m if u == 0 else None, False, {2: [prep_wot]} if u == 0 else {})

    def epi_body(ob, carry):
        qb = (ob * OB) // MQ
        lanes = pl.ds(pl.multiple_of((ob * OB) % MQ, OB), OB)
        cols = pl.ds(pl.multiple_of(ob * OB, OB), OB)
        oc = jnp.concatenate([ot_s[qb, h * VR:h * VR + DH, lanes] for h in range(H)],
                             axis=0).astype(BF16)
        bo = jnp.dot(wot_s[...], oc, preferred_element_type=F32)
        full = jnp.concatenate([at_s[:, cols], bo], axis=0)
        ob_s[cols, 512:1152] = full.T.astype(BF16)
        out_copy_b(ob).start()
        return carry
    jax.lax.fori_loop(0, NOB, epi_body, 0)
    for j in range(NAB):
        out_copy_a(j).wait()
    for ob in range(NOB):
        out_copy_b(ob).wait()


@jax.jit
def pallas_concat_heads__spectral_gfnet__mha_block__prompt_kernel(
    A_x: jax.Array,
    A_w_r: jax.Array,
    A_w_i: jax.Array,
    B_x: jax.Array,
    B_wqkv: jax.Array,
    B_wo: jax.Array,
):
    fa, fi2, cf, cb = _tables()
    fa = jnp.asarray(fa, BF16)
    fi2 = jnp.asarray(fi2, BF16)
    cf = jnp.asarray(cf, BF16)
    cb = jnp.asarray(cb, BF16)
    anyspec = pl.BlockSpec(memory_space=pl.ANY)
    out = pl.pallas_call(
        _kernel,
        out_shape=jax.ShapeDtypeStruct((S, 2 * D), BF16),
        in_specs=[anyspec] * 10,
        out_specs=anyspec,
        scratch_shapes=[
            pltpu.VMEM((D, S), BF16),
            pltpu.VMEM((DF, S), BF16),
            pltpu.VMEM((DF, S), BF16),
            pltpu.VMEM((D, S), BF16),
            pltpu.VMEM((D, 3 * D), BF16),
            pltpu.VMEM((D, D), BF16),
            pltpu.VMEM((NT, 2 * TR, DH2), BF16),
            pltpu.VMEM((2, DH2, 4 * TR), BF16),
            pltpu.VMEM((N1, 2 * N2, 2 * N2), BF16),
            pltpu.VMEM((N1, 2 * N2, 2 * N2), BF16),
            pltpu.SemaphoreType.DMA((9,)),
            pltpu.SemaphoreType.DMA((NPB,)),
            pltpu.SemaphoreType.DMA((NAB,)),
            pltpu.SemaphoreType.DMA((NOB,)),
            pltpu.VMEM((2, DH2, S), BF16),
            pltpu.VMEM((2 * TR, S), F32),
            pltpu.VMEM((N1, TR, 2 * N2), F32),
            pltpu.VMEM((N1, TR, 2 * N2), BF16),
            pltpu.VMEM((3, S, 128), jnp.int32),
            pltpu.VMEM((N1, 384, 128), jnp.int32),
            pltpu.VMEM((2, 4 * TR, S), F32),
            pltpu.VMEM((64, S), F32),
            pltpu.VMEM((1280 + D, D), F32),
            pltpu.VMEM((1280 + D, D), BF16),
            pltpu.VMEM((D, D), BF16),
            pltpu.VMEM((NG, S, 128), BF16),
            pltpu.VMEM((NQ, NG * 128, MQ), BF16),
            pltpu.VMEM((H * VR, S), BF16),
            pltpu.VMEM((NQ, H * VR, MQ), F32),
            pltpu.VMEM((S, MQ), F32),
            pltpu.VMEM((S, MQ), F32),
            pltpu.VMEM((S, 2 * D), BF16),
        ],
        compiler_params=pltpu.CompilerParams(vmem_limit_bytes=120 * 1024 * 1024),
    )(A_x[0].T, A_w_r.T, A_w_i.T, B_x[0].T, B_wqkv, B_wo, fa, fi2, cf, cb)
    return out.reshape(1, S, 2 * D)
```

```python
import functools

import numpy as np
import jax
import jax.numpy as jnp
from jax.experimental import pallas as pl
from jax.experimental.pallas import tpu as pltpu

S, D, H, DH = 2048, 576, 32, 18
DF = D // 2 + 1
DH2 = D // 2
TR = 80
NT = 4
HPG = 7
NG = 5
GW = HPG * DH
VR = 24
N1, N2 = 16, 128
MQ = 512
KC = 128
WM = 0.3
UNR = 4
NQ = S // MQ
NC = S // KC
PB = 256
NPB = S // PB
AB = 512
NAB = S // AB
OB = 512
NOB = S // OB
SL_A1, SL_FF, SL_M1, SL_M2, SL_FI = 0, 11, 24, 28, 48
QR = 4 * 128 + 80
WLR = 2 * QR + D
QSCALE = float(DH ** -0.5 * np.log2(np.e))
F32 = jnp.float32
BF16 = jnp.bfloat16
U32 = jnp.uint32


def _tables():
    d = np.arange(DH2)[None, :].astype(np.float64)
    fa = np.zeros((NT, 2 * TR, DH2), np.float64)
    fi2 = np.zeros((2, DH2, 4 * TR), np.float64)
    for c in range(NT):
        p, half = c // 2, c % 2
        l = p + 2 * (TR * half + np.arange(TR))
        valid = (l <= DF - 1).astype(np.float64)[:, None]
        lf = l[:, None].astype(np.float64)
        ang = 2.0 * np.pi * ((lf * d) % D) / D
        fa[c, :TR] = np.cos(ang) * valid
        fa[c, TR:] = -np.sin(ang) * valid
        cl = np.where((l == 0) | (l == DF - 1), 1.0, 2.0)[:, None] * valid
        im_ok = ((l != 0) & (l != DF - 1)).astype(np.float64)[:, None]
        fi2[p, :, half * 2 * TR:half * 2 * TR + TR] = (cl * np.cos(ang)).T / (S * D)
        fi2[p, :, half * 2 * TR + TR:(half + 1) * 2 * TR] = (-cl * im_ok * np.sin(ang)).T / (S * D)
    n2 = np.arange(N2)[:, None]
    k2 = np.arange(N2)[None, :]
    cf = np.zeros((N1, 2 * N2, 2 * N2), np.float64)
    for k1 in range(N1):
        th = 2.0 * np.pi * ((n2 * (k1 + N1 * k2)) % S) / S
        cr, ci = np.cos(th), -np.sin(th)
        cf[k1, :N2, :N2] = cr
        cf[k1, :N2, N2:] = ci
        cf[k1, N2:, :N2] = -ci
        cf[k1, N2:, N2:] = cr
    cb = np.ascontiguousarray(np.transpose(cf, (0, 2, 1)))
    return (fa.astype(np.float32), fi2.astype(np.float32),
            cf.astype(np.float32), cb.astype(np.float32))


def _cmul_const(xr, xi, k, n, sign):
    k = k % n
    if k == 0:
        return xr, xi
    if 4 * k == n:
        return (-xi, xr) if sign > 0 else (xi, -xr)
    if 2 * k == n:
        return -xr, -xi
    if 4 * k == 3 * n:
        return (xi, -xr) if sign > 0 else (-xi, xr)
    c = float(np.cos(2 * np.pi * k / n))
    s = float(sign * np.sin(2 * np.pi * k / n))
    if abs(abs(c) - abs(s)) < 1e-12:
        if c * s > 0:
            return (xr - xi) * c, (xr + xi) * c
        return (xr + xi) * c, (xi - xr) * c
    return xr * c - xi * s, xr * s + xi * c


def _fft(xs, sign):
    n = len(xs)
    if n == 1:
        return xs
    ev = _fft(xs[0::2], sign)
    od = _fft(xs[1::2], sign)
    out = [None] * n
    for k in range(n // 2):
        tr, ti = _cmul_const(od[k][0], od[k][1], k, n, sign)
        er, ei = ev[k]
        out[k] = (er + tr, ei + ti)
        out[k + n // 2] = (er - tr, ei - ti)
    return out


def _kernel(axt_hbm, wrt_hbm, wit_hbm, bxt_hbm, wqkv_hbm, wo_hbm,
            fa_hbm, fi_hbm, cf_hbm, cb_hbm, o_hbm,
            axt, wrt, wit, bxt, wqkv, wo, fa, fi2, cf, cb, sems, wsem, bsem, osem, osem2,
            xs_s, y_s, t_s, u_s, wn_s, wq_s, yb_s, at_s,
            wl_s, wl_b, wot_s, k_s, qt_s, vt_s, ot_s, sa, sb, ob_s):
    names = ["wrt", "wit", "axt", "fa", "cf", "cb", "fi", "wo"]
    srcs = [wrt_hbm, wit_hbm, axt_hbm, fa_hbm, cf_hbm, cb_hbm, fi_hbm, wo_hbm]
    dsts = [wrt, wit, axt, fa, cf, cb, fi2, wo]
    cp = {n_: pltpu.make_async_copy(s_, d_, sems.at[i])
          for i, (n_, s_, d_) in enumerate(zip(names, srcs, dsts))}

    def bx_copy(i):
        cols = pl.ds(pl.multiple_of(i * PB, PB), PB)
        return pltpu.make_async_copy(bxt_hbm.at[:, cols], bxt.at[:, cols], bsem.at[i])

    wch = [(0, 640), (640, 1280), (1280, 3 * D)]
    wcp = [pltpu.make_async_copy(wqkv_hbm.at[:, pl.ds(a_, b_ - a_)], wqkv.at[:, pl.ds(a_, b_ - a_)],
                                 wsem.at[i]) for i, (a_, b_) in enumerate(wch)]
    for c_ in wcp:
        c_.start()
    bx_copy(0).start()

    segs = []
    for g in range(NG):
        w = min(GW, D - g * GW)
        segs.append((g * 128, g * GW, w))
        segs.append((QR + g * 128, D + g * GW, w))
    segs.append((2 * QR, 2 * D, D))
    wl_s[...] = jnp.zeros(wl_s.shape, F32)
    for i, (a_, b_) in enumerate(wch):
        wcp[i].wait()
        if i == 0:
            for i_ in range(1, NPB):
                bx_copy(i_).start()
            for n_ in names:
                cp[n_].start()
        wt = wqkv[:, a_:b_].astype(F32).T
        for dr, sr, ln in segs:
            lo, hi = max(sr, a_), min(sr + ln, b_)
            if lo < hi:
                wl_s[dr + lo - sr:dr + hi - sr, :] = wt[lo - a_:hi - a_, :]
    wl_b[0:WLR, :] = wl_s[...].astype(BF16)

    def proj_block(cbk):
        bx_copy(cbk).wait()
        c0 = pl.multiple_of(cbk * PB, PB)
        cols = pl.ds(c0, PB)
        pr = jnp.dot(wl_b[0:WLR, :], bxt[:, cols], preferred_element_type=F32)
        zpad = jnp.zeros((NG * 128 - QR, PB), F32)
        qt = jnp.concatenate([pr[:QR, :] * QSCALE, zpad], axis=0)
        qlanes = pl.ds(pl.multiple_of((cbk * PB) % MQ, PB), PB)
        rid = jax.lax.broadcasted_iota(jnp.int32, (128, PB), 0)
        for h in range(H):
            g, j = h // HPG, h % HPG
            qg = qt[g * 128:(g + 1) * 128, :]
            qm = jnp.where((rid >= j * DH) & (rid < j * DH + DH), qg, 0.0)
            qt_s[(cbk * PB) // MQ, h, :, qlanes] = pltpu.bitcast(qm.astype(BF16), U32)
        kt = jnp.concatenate([pr[QR:2 * QR, :], zpad], axis=0).T.astype(BF16)
        krows = pl.ds(pl.multiple_of(cbk * (PB // 2), PB // 2), PB // 2)
        for g in range(NG):
            k_s[g, krows, :] = pltpu.bitcast(kt[:, g * 128:(g + 1) * 128], U32)
        vt = pr[2 * QR:, :]
        pad = jnp.concatenate([jnp.ones((1, PB), F32), jnp.zeros((VR - DH - 1, PB), F32)], axis=0)
        for h in range(H):
            blk = jnp.concatenate([vt[h * DH:(h + 1) * DH, :], pad], axis=0)
            vt_s[h * VR:(h + 1) * VR, cols] = blk.astype(BF16).astype(F32)

    def wperm1(c):
        l0 = pl.multiple_of(c * 128, 128)
        hi = pltpu.bitcast(wrt[:, pl.ds(l0, 128)].astype(F32), jnp.int32)
        lo = pltpu.bitcast(wit[:, pl.ds(l0, 128)].astype(F32), jnp.int32)
        blk = hi | jax.lax.shift_right_logical(lo, 16)
        blk = jnp.concatenate([blk, jnp.zeros((384 - DF, 128), jnp.int32)], axis=0)
        bt = blk.T
        for j in range(3):
            wn_s[j, pl.ds(l0, 128), :] = bt[:, j * 128:(j + 1) * 128]

    def wperm2(k1):
        for j in range(3):
            wq_s[k1, j * 128:(j + 1) * 128, :] = wn_s[j, pl.ds(k1, N2, stride=N1), :].T

    HP = NPB // 2

    def proj_a(i, carry):
        proj_block(i)
        return carry
    jax.lax.fori_loop(0, HP, proj_a, 0)

    cp["wrt"].wait()
    cp["wit"].wait()
    cp["axt"].wait()

    def proj_b(i, carry):
        proj_block(HP + i)
        for cc in range(N1 // HP):
            wperm1(i * (N1 // HP) + cc)
        cols = pl.ds(pl.multiple_of(i * (S // HP), S // HP), S // HP)
        x0 = axt[0:DH2, cols].astype(F32)
        x1 = axt[DH2:D, cols].astype(F32)
        xs_s[0, :, cols] = (x0 + x1).astype(BF16)
        xs_s[1, :, cols] = (x0 - x1).astype(BF16)
        return carry
    jax.lax.fori_loop(0, HP, proj_b, 0)

    cp["wo"].wait()
    cp["fa"].wait()
    cp["cf"].wait()
    cp["cb"].wait()
    cp["fi"].wait()

    def task_ops(c):
        p = c // 2
        half = c % 2
        sched = {}

        def put(slot, op):
            sched.setdefault(slot, []).append(op)

        def a1(j):
            cols = slice(j * 256, (j + 1) * 256)
            y_s[:, cols] = jnp.dot(fa[c], xs_s[p, :, cols], preferred_element_type=F32)
        for j in range(8):
            put(SL_A1 + j, functools.partial(a1, j))

        def ffwd(rc):
            rr = rc * 8
            xs = [(y_s[rr:rr + 8, n1 * 128:(n1 + 1) * 128],
                   y_s[TR + rr:TR + rr + 8, n1 * 128:(n1 + 1) * 128]) for n1 in range(N1)]
            out = _fft(xs, -1)
            for k1 in range(N1):
                t_s[k1, rr:rr + 8, 0:128] = out[k1][0]
                t_s[k1, rr:rr + 8, 128:256] = out[k1][1]
        for rc in range(TR // 8):
            put(SL_FF + rc, functools.partial(ffwd, rc))

        def mid1(k1):
            xk = jnp.dot(t_s[k1].astype(BF16), cf[k1], preferred_element_type=F32)
            xr, xi = xk[:, :128], xk[:, 128:]
            r0 = p + 2 * TR * half
            wp = wq_s[k1, pl.ds(r0, TR, stride=2), :]
            wr = pltpu.bitcast(wp & jnp.int32(-65536), F32)
            wi = pltpu.bitcast(jax.lax.shift_left(wp, 16), F32)
            u_s[k1] = jnp.concatenate([xr * wr - xi * wi, xr * wi + xi * wr], axis=1).astype(BF16)

        def mid2(k1):
            vk = jnp.dot(u_s[k1], cb[k1], preferred_element_type=F32)
            y_s[0:TR, k1 * 128:(k1 + 1) * 128] = vk[:, :128]
            y_s[TR:2 * TR, k1 * 128:(k1 + 1) * 128] = vk[:, 128:]
        for k1 in range(N1):
            put(SL_M1 + k1, functools.partial(mid1, k1))
            put(SL_M2 + k1, functools.partial(mid2, k1))

        def finv(rc):
            rr = rc * 8
            xs = [(y_s[rr:rr + 8, k1 * 128:(k1 + 1) * 128],
                   y_s[TR + rr:TR + rr + 8, k1 * 128:(k1 + 1) * 128]) for k1 in range(N1)]
            out = _fft(xs, +1)
            b0 = pl.multiple_of(half * 2 * TR + rr, 8)
            b1 = pl.multiple_of(half * 2 * TR + TR + rr, 8)
            for n1 in range(N1):
                yb_s[p, pl.ds(b0, 8), n1 * 128:(n1 + 1) * 128] = out[n1][0]
                yb_s[p, pl.ds(b1, 8), n1 * 128:(n1 + 1) * 128] = out[n1][1]
        for rc in range(TR // 8):
            put(SL_FI + rc, functools.partial(finv, rc))
        return sched

    def out_copy_a(j):
        rows = pl.ds(pl.multiple_of(j * AB, AB), AB)
        return pltpu.make_async_copy(ob_s.at[rows, pl.ds(0, 512)], o_hbm.at[rows, pl.ds(0, 512)],
                                     osem.at[j])

    def out_copy_b(ob):
        rows = pl.ds(pl.multiple_of(ob * OB, OB), OB)
        return pltpu.make_async_copy(ob_s.at[rows, pl.ds(512, 640)], o_hbm.at[rows, pl.ds(512, 640)],
                                     osem2.at[ob])

    def a7_ops(j):
        def one(q):
            cols = pl.ds(pl.multiple_of(j * AB + q * 128, 128), 128)
            e = jnp.dot(fi2[0], yb_s[0, :, cols].astype(BF16), preferred_element_type=F32)
            o = jnp.dot(fi2[1], yb_s[1, :, cols].astype(BF16), preferred_element_type=F32)
            ao = jnp.concatenate([e + o, e - o], axis=0)
            ob_s[cols, 0:512] = ao[:512].T.astype(BF16)
            at_s[:, cols] = ao[512:]
        return {4 + 14 * q: [functools.partial(one, q)] for q in range(AB // 128)}

    def step(t_qk, s_w, t_sm, s_r, m_in, want_m, extra={}):
        st = {}
        qk_ops = []
        if t_qk is not None:
            hq = t_qk // NQ
            qbq = t_qk % NQ
            g = hq // HPG
            st["mw"] = None

            def qk_c(c):
                kk = pltpu.bitcast(k_s[g, c * (KC // 2):(c + 1) * (KC // 2), :], BF16)
                qm = pltpu.bitcast(qt_s[qbq, hq], BF16)
                s = jnp.dot(kk, qm, preferred_element_type=F32)
                s_w[c * KC:(c + 1) * KC, :] = s
                if want_m:
                    m = jnp.max(s.reshape(KC // 8, 8, MQ), axis=0)
                    st["mw"] = m if st["mw"] is None else jnp.maximum(st["mw"], m)
            qk_ops = [functools.partial(qk_c, c) for c in range(NC)]
        sm_ops = []
        if t_sm is not None:
            h = t_sm // NQ
            qb = t_sm % NQ
            hv = h * VR if isinstance(h, int) else pl.multiple_of(h * VR, 8)
            st["mx"] = None
            st["acc"] = None
            st["m"] = m_in

            def mx_c(c):
                m = jnp.max(s_r[c * KC:(c + 1) * KC, :].reshape(KC // 8, 8, MQ), axis=0)
                st["mx"] = m if st["mx"] is None else jnp.maximum(st["mx"], m)
                if c == NC - 1:
                    st["m"] = jnp.max(st["mx"], axis=0, keepdims=True)

            def ex_c(c):
                p = jnp.exp2(s_r[c * KC:(c + 1) * KC, :] - st["m"]).astype(BF16)
                v = vt_s[pl.ds(hv, VR), c * KC:(c + 1) * KC]
                o = jnp.dot(v, p, preferred_element_type=F32)
                st["acc"] = o if st["acc"] is None else st["acc"] + o
                if c == NC - 1:
                    acc = st["acc"]
                    l = acc[DH:DH + 1, :]
                    ot_s[qb, pl.ds(hv, VR), :] = acc * (1.0 / l)
            if m_in is None:
                sm_ops = [(WM, functools.partial(mx_c, c)) for c in range(NC)]
            sm_ops += [(1.0, functools.partial(ex_c, c)) for c in range(NC)]
        tot = sum(w for w, _ in sm_ops)
        k = 0
        cum = 0.0
        for i, q in enumerate(qk_ops):
            q()
            while k < len(sm_ops) and cum + sm_ops[k][0] <= tot * (i + 1) / len(qk_ops) + 1e-9:
                cum += sm_ops[k][0]
                sm_ops[k][1]()
                k += 1
            for op in extra.get(i, ()):
                op()
        while k < len(sm_ops):
            sm_ops[k][1]()
            k += 1
        if want_m:
            return jnp.max(st["mw"], axis=0, keepdims=True)

    T = H * NQ
    bufs = [sa, sb]
    m0 = step(0, sa, None, None, None, True,
              {k1: [functools.partial(wperm2, k1)] for k1 in range(N1)})
    nb = (T - 1) // UNR

    def make_body(extra_fn, post_fn=None):
        def body(i, m):
            t = UNR * i
            ex = extra_fn(i) if extra_fn is not None else {}
            mm = None
            for u in range(UNR):
                part = {sl - u * NC: ops for sl, ops in ex.items() if u * NC <= sl < (u + 1) * NC}
                mm = step(t + u + 1, bufs[(u + 1) % 2], t + u, bufs[u % 2],
                          m if u == 0 else None, u == UNR - 1, part)
            if post_fn is not None:
                post_fn(i)
            return mm
        return body

    m = jax.lax.fori_loop(0, NT, make_body(task_ops), m0)
    m = jax.lax.fori_loop(NT, NT + NAB, make_body(lambda i: a7_ops(i - NT),
                                                  lambda i: out_copy_a(i - NT).start()), m)
    m = jax.lax.fori_loop(NT + NAB, nb, make_body(None), m)
    t0 = nb * UNR
    def prep_wot():
        wot_s[...] = wo[...].astype(F32).T.astype(BF16)

    for t in range(t0, T):
        u = t - t0
        step(t + 1 if t + 1 < T else None, bufs[(u + 1) % 2], t, bufs[u % 2],
             m if u == 0 else None, False, {2: [prep_wot]} if u == 0 else {})

    def epi_body(ob, carry):
        qb = (ob * OB) // MQ
        lanes = pl.ds(pl.multiple_of((ob * OB) % MQ, OB), OB)
        cols = pl.ds(pl.multiple_of(ob * OB, OB), OB)
        oc = jnp.concatenate([ot_s[qb, h * VR:h * VR + DH, lanes] for h in range(H)],
                             axis=0).astype(BF16)
        bo = jnp.dot(wot_s[...], oc, preferred_element_type=F32)
        full = jnp.concatenate([at_s[:, cols], bo], axis=0)
        ob_s[cols, 512:1152] = full.T.astype(BF16)
        out_copy_b(ob).start()
        return carry
    jax.lax.fori_loop(0, NOB, epi_body, 0)
    for j in range(NAB):
        out_copy_a(j).wait()
    for ob in range(NOB):
        out_copy_b(ob).wait()


@jax.jit
def pallas_concat_heads__spectral_gfnet__mha_block__prompt_kernel(
    A_x: jax.Array,
    A_w_r: jax.Array,
    A_w_i: jax.Array,
    B_x: jax.Array,
    B_wqkv: jax.Array,
    B_wo: jax.Array,
):
    fa, fi2, cf, cb = _tables()
    fa = jnp.asarray(fa, BF16)
    fi2 = jnp.asarray(fi2, BF16)
    cf = jnp.asarray(cf, BF16)
    cb = jnp.asarray(cb, BF16)
    anyspec = pl.BlockSpec(memory_space=pl.ANY)
    out = pl.pallas_call(
        _kernel,
        out_shape=jax.ShapeDtypeStruct((S, 2 * D), BF16),
        in_specs=[anyspec] * 10,
        out_specs=anyspec,
        scratch_shapes=[
            pltpu.VMEM((D, S), BF16),
            pltpu.VMEM((DF, S), BF16),
            pltpu.VMEM((DF, S), BF16),
            pltpu.VMEM((D, S), BF16),
            pltpu.VMEM((D, 3 * D), BF16),
            pltpu.VMEM((D, D), BF16),
            pltpu.VMEM((NT, 2 * TR, DH2), BF16),
            pltpu.VMEM((2, DH2, 4 * TR), BF16),
            pltpu.VMEM((N1, 2 * N2, 2 * N2), BF16),
            pltpu.VMEM((N1, 2 * N2, 2 * N2), BF16),
            pltpu.SemaphoreType.DMA((8,)),
            pltpu.SemaphoreType.DMA((3,)),
            pltpu.SemaphoreType.DMA((NPB,)),
            pltpu.SemaphoreType.DMA((NAB,)),
            pltpu.SemaphoreType.DMA((NOB,)),
            pltpu.VMEM((2, DH2, S), BF16),
            pltpu.VMEM((2 * TR, S), F32),
            pltpu.VMEM((N1, TR, 2 * N2), F32),
            pltpu.VMEM((N1, TR, 2 * N2), BF16),
            pltpu.VMEM((3, S, 128), jnp.int32),
            pltpu.VMEM((N1, 384, 128), jnp.int32),
            pltpu.VMEM((2, 4 * TR, S), F32),
            pltpu.VMEM((64, S), F32),
            pltpu.VMEM((WLR, D), F32),
            pltpu.VMEM((1792, D), BF16),
            pltpu.VMEM((D, D), BF16),
            pltpu.VMEM((NG, S // 2, 128), U32),
            pltpu.VMEM((NQ, H, 64, MQ), U32),
            pltpu.VMEM((H * VR, S), F32),
            pltpu.VMEM((NQ, H * VR, MQ), F32),
            pltpu.VMEM((S, MQ), F32),
            pltpu.VMEM((S, MQ), F32),
            pltpu.VMEM((S, 2 * D), BF16),
        ],
        compiler_params=pltpu.CompilerParams(vmem_limit_bytes=120 * 1024 * 1024),
    )(A_x[0].T, A_w_r.T, A_w_i.T, B_x[0].T, B_wqkv, B_wo, fa, fi2, cf, cb)
    return out.reshape(1, S, 2 * D)
```
